```python
import jax
import jax.numpy as jnp

def _softmax(x, axis=-1):
    return jax.nn.softmax(x, axis=axis)
def _gelu(x):
    return jax.nn.gelu(x, approximate=True)
def _silu(x):
    return jax.nn.silu(x)
def _sigmoid(x):
    return jax.nn.sigmoid(x)
def _layernorm(x, axis=-1, eps=1e-5):
    m = jnp.mean(x, axis=axis, keepdims=True)
    v = jnp.var(x, axis=axis, keepdims=True)
    return (x - m) / jnp.sqrt(v + eps)
def _scatter_add(tgt, idx, src, axis=0):
    return tgt.at[idx].add(src)
def _segment_sum(src, seg, n):
    return jax.ops.segment_sum(src, seg, n)
class _Rng:
    def __init__(self, key):
        self._k = key
    def _next(self):
        self._k, sub = jax.random.split(self._k)
        return sub
    def normal(self, shape):
        return jax.random.normal(self._next(), shape, dtype=jnp.bfloat16)
    def randint(self, lo, hi, shape):
        return jax.random.randint(self._next(), shape, lo, hi, dtype=jnp.int32)
    def uniform(self, shape, lo=0.0, hi=1.0):
        return jax.random.uniform(self._next(), shape, jnp.bfloat16, lo, hi)
    def permutation(self, n):
        return jax.random.permutation(self._next(), n)


kernel_name = 'parallel_sum__sliding_block_cached__glu_gated_swiglu__decode'

def setup_inputs():
    _rng = _Rng(jax.random.key(int.from_bytes(__import__("os").urandom(4), "little")))
    _w = (lambda a: (lambda t: t.astype(jnp.bfloat16) if jnp.issubdtype(t.dtype, jnp.floating) else t)(jnp.asarray(a)))
    def _A_setup():
        B, Sq, D = 4, 1, 640
        Hq, Hkv, Sk, Dh = 32, 32, 8192, 192
        assert Hq % Hkv == 0, (Hq, Hkv)
        return {
            "x": _w((lambda *s: _rng.normal(s) * 0.05)(B, Sq, D)),
            "k_cache": _w((lambda *s: _rng.normal(s) * 0.05)(B, Hkv, Sk, Dh)),
            "v_cache": _w((lambda *s: _rng.normal(s) * 0.05)(B, Hkv, Sk, Dh)),
            "wq": _w((lambda *s: _rng.normal(s) * 0.05)(D, Hq * Dh) * (D ** -0.5)),
            "wo": _w((lambda *s: _rng.normal(s) * 0.05)(Hq * Dh, D) * ((Hq * Dh) ** -0.5)),
        }
    _A_in = _A_setup()

    def _B_setup():
        B, S, D, F = 4, 1, 640, 1536
        return {
            "x": _w((lambda *s: _rng.normal(s) * 0.05)(B, S, D)),
            "w1": _w((lambda *s: _rng.normal(s) * 0.05)(D, F) * (2.0 / D) ** 0.5),
            "w3": _w((lambda *s: _rng.normal(s) * 0.05)(D, F) * (2.0 / D) ** 0.5),
            "w2": _w((lambda *s: _rng.normal(s) * 0.05)(F, D) * (2.0 / F) ** 0.5),
        }
    _B_in = _B_setup()

    return {
        "A_x": _A_in["x"],
        "A_k_cache": _A_in["k_cache"],
        "A_v_cache": _A_in["v_cache"],
        "A_wq": _A_in["wq"],
        "A_wo": _A_in["wo"],
        "B_x": _B_in["x"],
        "B_w1": _B_in["w1"],
        "B_w3": _B_in["w3"],
        "B_w2": _B_in["w2"],
    }

def reference(A_x, A_k_cache, A_v_cache, A_wq, A_wo, B_x, B_w1, B_w3, B_w2):
    def _A_ref(x, k_cache, v_cache, wq, wo):
        B, Sq, D = x.shape
        Hq, Dh = 32, 192
        Hkv, Sk = k_cache.shape[1], k_cache.shape[2]
        W = min(4096, max(256, Sk // 4))
        rep = Hq // Hkv
        q = (lambda x, *d: x.transpose(*d))((x @ wq).reshape(B, Sq, Hq, Dh), 0, 2, 1, 3)
        k = jnp.repeat(k_cache[:, :, Sk - W:, :], rep, axis=1)
        v = jnp.repeat(v_cache[:, :, Sk - W:, :], rep, axis=1)
        scores = jnp.einsum("bhqd,bhkd->bhqk", q, k) * (Dh ** -0.5)
        p = _softmax(scores, axis=-1)
        o = jnp.einsum("bhqk,bhkd->bhqd", p, v)
        return (lambda x, *d: x.transpose(*d))(o, 0, 2, 1, 3).reshape(B, Sq, Hq * Dh) @ wo

    def _B_ref(x, w1, w3, w2):
        gate = jnp.einsum("bsd,df->bsf", x, w1)
        up = jnp.einsum("bsd,df->bsf", x, w3)
        h = _silu(gate) * up
        out = jnp.einsum("bsf,fd->bsd", h, w2)
        return out

    x = A_x
    xn = _layernorm(x, axis=-1)
    return x + _A_ref(xn, A_k_cache, A_v_cache, A_wq, A_wo) + _B_ref(xn, B_w1, B_w3, B_w2)
```

```python
import functools

import jax
import jax.numpy as jnp
import jax.experimental.pallas as pl
import jax.experimental.pallas.tpu as pltpu

_HQ, _DH = 32, 192
_HP = 2
_NSLOT = 3
_RSPLIT = 1


def _kernel(x_ref, k_hbm, v_hbm, wq_hbm, wo_hbm, w1_hbm, w3_hbm, w2_hbm, o_ref,
            kbuf, vbuf, wq_v, wo_v, w1_v, w3_v, w2_v, q_scr, ksem, vsem, wsem,
            *, B, W, Sk, D):
    NG = _HQ // _HP
    GW = _HP * _DH
    R = B * _HP
    f32, bf16 = jnp.float32, jnp.bfloat16

    def kv_copies(src, buf, sem, g, slot, b):
        out = []
        rr = _DH // _RSPLIT
        for hh in range(_HP):
            for s in range(_RSPLIT):
                out.append(pltpu.make_async_copy(
                    src.at[b, g * _HP + hh, pl.ds(s * rr, rr), pl.ds(Sk - W, W)],
                    buf.at[slot, b, pl.ds(hh * _DH + s * rr, rr), :],
                    sem.at[slot, b]))
        return out

    def kv_start(src, buf, sem, g, slot, b):
        for n, c in enumerate(kv_copies(src, buf, sem, g, slot, b)):
            c.start(priority=n % 2)

    def kv_wait(buf, sem, slot, b):
        pltpu.make_async_copy(buf.at[slot, b], buf.at[slot, b], sem.at[slot, b]).wait()

    wq_c = pltpu.make_async_copy(wq_hbm, wq_v, wsem.at[0])
    w1_c = pltpu.make_async_copy(w1_hbm, w1_v, wsem.at[1])
    w3_c = pltpu.make_async_copy(w3_hbm, w3_v, wsem.at[2])
    w2_c = pltpu.make_async_copy(w2_hbm, w2_v, wsem.at[3])
    wo_c = pltpu.make_async_copy(wo_hbm, wo_v, wsem.at[4])

    wq_c.start()
    for g in range(_NSLOT):
        for b in range(B):
            kv_start(k_hbm, kbuf, ksem, g, g, b)
        if g == 0:
            wo_c.start()
        for b in range(B):
            kv_start(v_hbm, vbuf, vsem, g, g, b)
    w1_c.start()
    w3_c.start()
    w2_c.start()

    x = x_ref[...].astype(f32)
    row = jax.lax.broadcasted_iota(jnp.int32, (R, D), 0)
    x8 = jnp.zeros((R, D), f32)
    for b in range(B):
        x8 = jnp.where(row // _HP == b, x[b:b + 1, :], x8)
    m = jnp.mean(x8, axis=-1, keepdims=True)
    xc = x8 - m
    var = jnp.mean(xc * xc, axis=-1, keepdims=True)
    xn = (xc / jnp.sqrt(var + 1e-5)).astype(bf16)

    wq_c.wait()
    q = jnp.dot(xn, wq_v[...], preferred_element_type=f32)
    q_scr[...] = q.astype(bf16).astype(f32) * (_DH ** -0.5)

    rowg = jax.lax.broadcasted_iota(jnp.int32, (R, GW), 0)
    colg = jax.lax.broadcasted_iota(jnp.int32, (R, GW), 1)
    own_head = (colg >= _DH).astype(jnp.int32) == rowg % _HP

    wo_c.wait()

    def body(g, acc):
        slot = g % _NSLOT
        qg = q_scr[:, pl.ds(pl.multiple_of(g * GW, 128), GW)]
        s = None
        for b in range(B):
            qb = jnp.where(own_head & (rowg // _HP == b), qg, 0.0).astype(bf16)
            kv_wait(kbuf, ksem, slot, b)
            sb = jnp.dot(qb, kbuf[slot, b], preferred_element_type=f32)
            s = sb if s is None else s + sb

        @pl.when(g + _NSLOT < NG)
        def _():
            for b in range(B):
                kv_start(k_hbm, kbuf, ksem, g + _NSLOT, slot, b)

        mx = jnp.max(s, axis=-1, keepdims=True)
        e = jnp.exp(s - mx)
        p = (e / jnp.sum(e, axis=-1, keepdims=True)).astype(bf16)
        o = jnp.zeros((R, GW), f32)
        for b in range(B):
            kv_wait(vbuf, vsem, slot, b)
            ob = jax.lax.dot_general(p, vbuf[slot, b], (((1,), (1,)), ((), ())),
                                     preferred_element_type=f32)
            o = jnp.where(own_head & (rowg // _HP == b), ob, o)

        @pl.when(g + _NSLOT < NG)
        def _():
            for b in range(B):
                kv_start(v_hbm, vbuf, vsem, g + _NSLOT, slot, b)

        wo_g = wo_v[pl.ds(pl.multiple_of(g * GW, 128), GW), :]
        return acc + jnp.dot(o.astype(bf16), wo_g, preferred_element_type=f32)

    acc = jax.lax.fori_loop(0, 2, body, jnp.zeros((R, D), f32))

    w1_c.wait()
    w3_c.wait()
    w2_c.wait()
    gate = jnp.dot(xn, w1_v[...], preferred_element_type=f32)
    up = jnp.dot(xn, w3_v[...], preferred_element_type=f32)
    hmid = (gate * jax.nn.sigmoid(gate) * up).astype(bf16)
    ffn = jnp.dot(hmid, w2_v[...], preferred_element_type=f32)

    acc = jax.lax.fori_loop(2, NG, body, acc)

    tot = acc + jnp.where(row % _HP == 0, x8 + ffn, 0.0)
    for b in range(B):
        o_ref[b:b + 1, :] = (tot[2 * b:2 * b + 1, :] + tot[2 * b + 1:2 * b + 2, :]).astype(o_ref.dtype)


@jax.jit
def pallas_parallel_sum__sliding_block_cached__glu_gated_swiglu__decode_kernel(
    A_x: jax.Array,
    A_k_cache: jax.Array,
    A_v_cache: jax.Array,
    A_wq: jax.Array,
    A_wo: jax.Array,
    B_x: jax.Array,
    B_w1: jax.Array,
    B_w3: jax.Array,
    B_w2: jax.Array,
):
    del B_x
    B, Sq, D = A_x.shape
    _, Hkv, Sk, Dh = A_k_cache.shape
    assert Sq == 1 and Hkv == _HQ and Dh == _DH and B * _HP == 8
    W = min(4096, max(256, Sk // 4))
    dt = A_k_cache.dtype

    kT = jnp.swapaxes(A_k_cache, 2, 3)
    vT = jnp.swapaxes(A_v_cache, 2, 3)
    hbm = pl.BlockSpec(memory_space=pl.ANY)
    out = pl.pallas_call(
        functools.partial(_kernel, B=B, W=W, Sk=Sk, D=D),
        out_shape=jax.ShapeDtypeStruct((B, D), A_x.dtype),
        in_specs=[pl.BlockSpec(memory_space=pltpu.VMEM)] + [hbm] * 7,
        out_specs=pl.BlockSpec(memory_space=pltpu.VMEM),
        scratch_shapes=[
            pltpu.VMEM((_NSLOT, B, _HP * Dh, W), dt),
            pltpu.VMEM((_NSLOT, B, _HP * Dh, W), dt),
            pltpu.VMEM(A_wq.shape, A_wq.dtype),
            pltpu.VMEM(A_wo.shape, A_wo.dtype),
            pltpu.VMEM(B_w1.shape, B_w1.dtype),
            pltpu.VMEM(B_w3.shape, B_w3.dtype),
            pltpu.VMEM(B_w2.shape, B_w2.dtype),
            pltpu.VMEM((B * _HP, _HQ * Dh), jnp.float32),
            pltpu.SemaphoreType.DMA((_NSLOT, B)),
            pltpu.SemaphoreType.DMA((_NSLOT, B)),
            pltpu.SemaphoreType.DMA((5,)),
        ],
        compiler_params=pltpu.CompilerParams(vmem_limit_bytes=100 * 1024 * 1024),
    )(A_x.reshape(B, D), kT, vT, A_wq, A_wo, B_w1, B_w3, B_w2)
    return out.reshape(B, Sq, D)
```

```python
import functools

import jax
import jax.numpy as jnp
import jax.experimental.pallas as pl
import jax.experimental.pallas.tpu as pltpu

_HQ, _DH = 32, 192
_HP = 2
_NSLOT = 1
_LSPLIT = 16


def _kernel(x_ref, k_hbm, v_hbm, wq_hbm, wo_hbm, w1_hbm, w3_hbm, w2_hbm, o_ref,
            kbuf, vbuf, wq_v, wo_v, w1_v, w3_v, w2_v, q_scr, ksem, vsem, wsem,
            *, B, W, Sk, D):
    NG = _HQ // _HP
    GW = _HP * _DH
    R = B * _HP
    f32, bf16 = jnp.float32, jnp.bfloat16

    def kv_start(src, buf, sem, g, slot, b):
        ww = W // _LSPLIT
        for l in range(_LSPLIT):
            pltpu.make_async_copy(
                src.at[b, pl.ds(g * _HP, _HP), :, pl.ds(Sk - W + l * ww, ww)],
                buf.at[slot, b, :, :, pl.ds(l * ww, ww)],
                sem.at[slot, b]).start(priority=l % 2)

    def kv_wait(buf, sem, slot, b):
        pltpu.make_async_copy(buf.at[slot, b], buf.at[slot, b], sem.at[slot, b]).wait()

    wq_c = pltpu.make_async_copy(wq_hbm, wq_v, wsem.at[0])
    w1_c = pltpu.make_async_copy(w1_hbm, w1_v, wsem.at[1])
    w3_c = pltpu.make_async_copy(w3_hbm, w3_v, wsem.at[2])
    w2_c = pltpu.make_async_copy(w2_hbm, w2_v, wsem.at[3])
    wo_c = pltpu.make_async_copy(wo_hbm, wo_v, wsem.at[4])

    wq_c.start()
    for g in range(_NSLOT):
        for b in range(B):
            kv_start(k_hbm, kbuf, ksem, g, g, b)
        if g == 0:
            wo_c.start()
        for b in range(B):
            kv_start(v_hbm, vbuf, vsem, g, g, b)
    w1_c.start()
    w3_c.start()
    w2_c.start()

    x = x_ref[...].astype(f32)
    row = jax.lax.broadcasted_iota(jnp.int32, (R, D), 0)
    x8 = jnp.zeros((R, D), f32)
    for b in range(B):
        x8 = jnp.where(row // _HP == b, x[b:b + 1, :], x8)
    m = jnp.mean(x8, axis=-1, keepdims=True)
    xc = x8 - m
    var = jnp.mean(xc * xc, axis=-1, keepdims=True)
    xn = (xc / jnp.sqrt(var + 1e-5)).astype(bf16)

    wq_c.wait()
    q = jnp.dot(xn, wq_v[...], preferred_element_type=f32)
    q_scr[...] = q.astype(bf16).astype(f32) * (_DH ** -0.5)

    rowg = jax.lax.broadcasted_iota(jnp.int32, (R, GW), 0)
    colg = jax.lax.broadcasted_iota(jnp.int32, (R, GW), 1)
    own_head = (colg >= _DH).astype(jnp.int32) == rowg % _HP

    wo_c.wait()

    def body(g, acc):
        slot = g % _NSLOT
        qg = q_scr[:, pl.ds(pl.multiple_of(g * GW, 128), GW)]
        s = None
        for b in range(B):
            qb = jnp.where(own_head & (rowg // _HP == b), qg, 0.0).astype(bf16)
            kv_wait(kbuf, ksem, slot, b)
            sb = jnp.dot(qb, kbuf[slot, b].reshape(GW, W), preferred_element_type=f32)
            s = sb if s is None else s + sb
            pl.when(g + _NSLOT < NG)(functools.partial(
                kv_start, k_hbm, kbuf, ksem, g + _NSLOT, slot, b))

        mx = jnp.max(s, axis=-1, keepdims=True)
        e = jnp.exp(s - mx)
        p = (e / jnp.sum(e, axis=-1, keepdims=True)).astype(bf16)
        o = jnp.zeros((R, GW), f32)
        for b in range(B):
            kv_wait(vbuf, vsem, slot, b)
            ob = jax.lax.dot_general(p, vbuf[slot, b].reshape(GW, W), (((1,), (1,)), ((), ())),
                                     preferred_element_type=f32)
            o = jnp.where(own_head & (rowg // _HP == b), ob, o)
            pl.when(g + _NSLOT < NG)(functools.partial(
                kv_start, v_hbm, vbuf, vsem, g + _NSLOT, slot, b))

        wo_g = wo_v[pl.ds(pl.multiple_of(g * GW, 128), GW), :]
        return acc + jnp.dot(o.astype(bf16), wo_g, preferred_element_type=f32)

    acc = jax.lax.fori_loop(0, 2, body, jnp.zeros((R, D), f32))

    w1_c.wait()
    w3_c.wait()
    w2_c.wait()
    gate = jnp.dot(xn, w1_v[...], preferred_element_type=f32)
    up = jnp.dot(xn, w3_v[...], preferred_element_type=f32)
    hmid = (gate * jax.nn.sigmoid(gate) * up).astype(bf16)
    ffn = jnp.dot(hmid, w2_v[...], preferred_element_type=f32)

    acc = jax.lax.fori_loop(2, NG, body, acc)

    tot = acc + jnp.where(row % _HP == 0, x8 + ffn, 0.0)
    for b in range(B):
        o_ref[b:b + 1, :] = (tot[2 * b:2 * b + 1, :] + tot[2 * b + 1:2 * b + 2, :]).astype(o_ref.dtype)


@jax.jit
def pallas_parallel_sum__sliding_block_cached__glu_gated_swiglu__decode_kernel(
    A_x: jax.Array,
    A_k_cache: jax.Array,
    A_v_cache: jax.Array,
    A_wq: jax.Array,
    A_wo: jax.Array,
    B_x: jax.Array,
    B_w1: jax.Array,
    B_w3: jax.Array,
    B_w2: jax.Array,
):
    del B_x
    B, Sq, D = A_x.shape
    _, Hkv, Sk, Dh = A_k_cache.shape
    assert Sq == 1 and Hkv == _HQ and Dh == _DH and B * _HP == 8
    W = min(4096, max(256, Sk // 4))
    dt = A_k_cache.dtype

    kT = jnp.swapaxes(A_k_cache, 2, 3)
    vT = jnp.swapaxes(A_v_cache, 2, 3)
    hbm = pl.BlockSpec(memory_space=pl.ANY)
    out = pl.pallas_call(
        functools.partial(_kernel, B=B, W=W, Sk=Sk, D=D),
        out_shape=jax.ShapeDtypeStruct((B, D), A_x.dtype),
        in_specs=[pl.BlockSpec(memory_space=pltpu.VMEM)] + [hbm] * 7,
        out_specs=pl.BlockSpec(memory_space=pltpu.VMEM),
        scratch_shapes=[
            pltpu.VMEM((_NSLOT, B, _HP, Dh, W), dt),
            pltpu.VMEM((_NSLOT, B, _HP, Dh, W), dt),
            pltpu.VMEM(A_wq.shape, A_wq.dtype),
            pltpu.VMEM(A_wo.shape, A_wo.dtype),
            pltpu.VMEM(B_w1.shape, B_w1.dtype),
            pltpu.VMEM(B_w3.shape, B_w3.dtype),
            pltpu.VMEM(B_w2.shape, B_w2.dtype),
            pltpu.VMEM((B * _HP, _HQ * Dh), jnp.float32),
            pltpu.SemaphoreType.DMA((_NSLOT, B)),
            pltpu.SemaphoreType.DMA((_NSLOT, B)),
            pltpu.SemaphoreType.DMA((5,)),
        ],
        compiler_params=pltpu.CompilerParams(vmem_limit_bytes=100 * 1024 * 1024),
    )(A_x.reshape(B, D), kT, vT, A_wq, A_wo, B_w1, B_w3, B_w2)
    return out.reshape(B, Sq, D)
```
